```python
import os as _os
_os.environ.setdefault("JAX_PLATFORMS", "cpu")
import jax
import jax.numpy as jnp

def _softmax(x, axis=-1):
    return jax.nn.softmax(x, axis=axis)
def _gelu(x):
    return jax.nn.gelu(x, approximate=True)
def _silu(x):
    return jax.nn.silu(x)
def _sigmoid(x):
    return jax.nn.sigmoid(x)
def _layernorm(x, axis=-1, eps=1e-5):
    m = jnp.mean(x, axis=axis, keepdims=True)
    v = jnp.var(x, axis=axis, keepdims=True)
    return (x - m) / jnp.sqrt(v + eps)
def _scatter_add(tgt, idx, src, axis=0):
    return tgt.at[idx].add(src)
def _segment_sum(src, seg, n):
    return jax.ops.segment_sum(src, seg, n)
class _Rng:
    def __init__(self, key):
        self._k = key
    def _next(self):
        self._k, sub = jax.random.split(self._k)
        return sub
    def normal(self, shape):
        return jax.random.normal(self._next(), shape, dtype=jnp.bfloat16)
    def randint(self, lo, hi, shape):
        return jax.random.randint(self._next(), shape, lo, hi, dtype=jnp.int32)
    def uniform(self, shape, lo=0.0, hi=1.0):
        return jax.random.uniform(self._next(), shape, jnp.bfloat16, lo, hi)
    def permutation(self, n):
        return jax.random.permutation(self._next(), n)


kernel_name = 'gated_mix__mha_block__mha_block__prompt'

def setup_inputs():
    _rng = _Rng(jax.random.key(int.from_bytes(__import__("os").urandom(4), "little")))
    _w = (lambda a: (lambda t: t.astype(jnp.bfloat16) if jnp.issubdtype(t.dtype, jnp.floating) else t)(jnp.asarray(a)))
    def _A_setup():
        B, S, D, H = 1, 2048, 448, 16
        return {
            "x": _w((lambda *s: _rng.normal(s) * 0.05)(B, S, D)),
            "wqkv": _w((lambda *s: _rng.normal(s) * 0.4)(D, 3 * D)),
            "wo": _w((lambda *s: _rng.normal(s) * 0.05)(D, D)),
        }
    _A_in = _A_setup()

    def _B_setup():
        B, S, D, H = 1, 2048, 448, 16
        return {
            "x": _w((lambda *s: _rng.normal(s) * 0.05)(B, S, D)),
            "wqkv": _w((lambda *s: _rng.normal(s) * 0.4)(D, 3 * D)),
            "wo": _w((lambda *s: _rng.normal(s) * 0.05)(D, D)),
        }
    _B_in = _B_setup()

    return {
        "A_x": _A_in["x"],
        "A_wqkv": _A_in["wqkv"],
        "A_wo": _A_in["wo"],
        "B_x": _B_in["x"],
        "B_wqkv": _B_in["wqkv"],
        "B_wo": _B_in["wo"],
        "gate_w": _w((lambda *s: _rng.normal(s) * 0.05)(448) * 16.0),
    }

def reference(A_x, A_wqkv, A_wo, B_x, B_wqkv, B_wo, gate_w):
    def _A_ref(x, wqkv, wo):
        B, S, D = x.shape
        H = 16
        Dh = D // H
        qkv = (lambda x, *d: x.transpose(*d))((x @ wqkv).reshape(B, S, 3, H, Dh), 2, 0, 3, 1, 4)
        q, k, v = qkv[0], qkv[1], qkv[2]
        scores = jnp.einsum("bhqd,bhkd->bhqk", q, k) * (Dh ** -0.5)
        p = _softmax(scores, axis=-1)
        o = jnp.einsum("bhqk,bhkd->bhqd", p, v)
        return (lambda x, *d: x.transpose(*d))(o, 0, 2, 1, 3).reshape(B, S, D) @ wo

    def _B_ref(x, wqkv, wo):
        B, S, D = x.shape
        H = 16
        Dh = D // H
        qkv = (lambda x, *d: x.transpose(*d))((x @ wqkv).reshape(B, S, 3, H, Dh), 2, 0, 3, 1, 4)
        q, k, v = qkv[0], qkv[1], qkv[2]
        scores = jnp.einsum("bhqd,bhkd->bhqk", q, k) * (Dh ** -0.5)
        p = _softmax(scores, axis=-1)
        o = jnp.einsum("bhqk,bhkd->bhqd", p, v)
        return (lambda x, *d: x.transpose(*d))(o, 0, 2, 1, 3).reshape(B, S, D) @ wo

    x = A_x
    g = _sigmoid((x * gate_w).sum(-1, keepdims=True))
    a = _A_ref(x, A_wqkv, A_wo)
    b = _B_ref(x, B_wqkv, B_wo)
    return g * a + (1 - g) * b
```

```python
import math

import jax
import jax.numpy as jnp
import jax.experimental.pallas as pl
import jax.experimental.pallas.tpu as pltpu

S = 2048
D = 448
H = 16
DH = D // H
G = 4
NG = H // G
BQ = 512
KC = 128
NQ = S // BQ
NHEADS = 2 * H
NIT = NHEADS * NQ
QSCALE = (DH ** -0.5) * math.log2(math.e)
BF = jnp.bfloat16
F32 = jnp.float32

_NT = (((1,), (1,)), ((), ()))


def _kernel(x_ref, wa_ref, woa_ref, wb_ref, wob_ref, gw_ref, o_ref,
            k_scr, q_scr, vt_scr, s0, s1, m0, m1, ot_scr):
    RC = 512
    for b, w_ref in enumerate((wa_ref, wb_ref)):
        for g in range(NG):
            wq = w_ref[:, g * G * DH: g * G * DH + 128]
            wk = w_ref[:, D + g * G * DH: D + g * G * DH + 128]
            wqk = jnp.concatenate([wq, wk], axis=1)
            for r in range(S // RC):
                xs = x_ref[r * RC:(r + 1) * RC, :]
                qk = jnp.dot(xs, wqk, preferred_element_type=F32)
                q_scr[b * NG + g, r * RC:(r + 1) * RC, :] = (qk[:, :128] * QSCALE).astype(BF)
                k_scr[b * NG + g, r * RC:(r + 1) * RC, :] = qk[:, 128:].astype(BF)
        wvt = w_ref[:, 2 * D:3 * D].astype(F32).T.astype(BF)
        vt = lax_dot_nt(wvt, x_ref[...])
        row = jax.lax.broadcasted_iota(jnp.int32, (32, S), 0)
        for h in range(H):
            if h < H - 1:
                vh = vt[h * DH: h * DH + 32, :]
            else:
                vh = jnp.concatenate([vt[h * DH:, :], jnp.zeros((32 - DH, S), F32)], axis=0)
            vh = jnp.where(row == DH, 1.0, vh)
            vt_scr[b * H + h] = vh.astype(BF)

    lane = jax.lax.broadcasted_iota(jnp.int32, (BQ, 128), 1)

    def step(itA, sA, mA, itB, sB, mB_ref, doA=True, doB=True):
        st = {}
        if doA:
            hA = itA // NQ
            qsA = pl.multiple_of((itA % NQ) * BQ, BQ)
            gA = hA // G
            lo = (hA % G) * DH
            q = q_scr[gA, pl.ds(qsA, BQ), :]
            qm = jnp.where((lane >= lo) & (lane < lo + DH), q, jnp.zeros_like(q))
            st['m'] = None
        if doB:
            hB = itB // NQ
            qsB = pl.multiple_of((itB % NQ) * BQ, BQ)
            mm = jnp.tile(mB_ref[...], (KC // 8, 1))
            st['acc'] = jnp.zeros((32, BQ), F32)

        def a(c):
            kk = k_scr[gA, c * KC:(c + 1) * KC, :]
            s = jax.lax.dot_general(kk, qm, _NT, preferred_element_type=F32)
            sA[c * KC:(c + 1) * KC, :] = s
            sm = s[0:8]
            for r in range(1, KC // 8):
                sm = jnp.maximum(sm, s[r * 8:(r + 1) * 8])
            st['m'] = sm if st['m'] is None else jnp.maximum(st['m'], sm)

        def b(c):
            s = sB[c * KC:(c + 1) * KC, :]
            p = jnp.exp2(s - mm).astype(BF)
            st['acc'] = st['acc'] + jnp.dot(vt_scr[hB, :, c * KC:(c + 1) * KC], p,
                                            preferred_element_type=F32)

        for c in range(S // KC):
            if doA:
                a(c)
            if doB:
                b(c)
        if doA:
            mA[...] = jnp.broadcast_to(jnp.max(st['m'], axis=0, keepdims=True), (8, BQ))
        if doB:
            acc = st['acc']
            l = acc[DH:DH + 1, :]
            o = acc * (1.0 / l)
            ot_scr[hB, :, pl.ds(qsB, BQ)] = o.astype(BF)

    step(0, s0, m0, None, None, None, True, False)

    def body(j, c):
        i = 2 * j
        step(i + 1, s1, m1, i, s0, m0)
        step(i + 2, s0, m0, i + 1, s1, m1)
        return c

    jax.lax.fori_loop(0, NIT // 2 - 1, body, 0)
    step(NIT - 1, s1, m1, NIT - 2, s0, m0)
    step(None, None, None, NIT - 1, s1, m1, False, True)

    gl = jax.lax.dot_general(jnp.broadcast_to(gw_ref[...], (8, D)), x_ref[...], _NT,
                             preferred_element_type=F32)[0:1, :]
    gate = 1.0 / (1.0 + jnp.exp(-gl))
    outs = []
    for b, wo_ref in enumerate((woa_ref, wob_ref)):
        wo = wo_ref[...]
        z = jnp.zeros((32 - DH, D), BF)
        wo_pad = jnp.concatenate(
            [t for h in range(H) for t in (wo[h * DH:(h + 1) * DH], z)], axis=0)
        wot = wo_pad.astype(F32).T.astype(BF)
        ot = ot_scr[b * H:(b + 1) * H].reshape(H * 32, S)
        outs.append(jnp.dot(wot, ot, preferred_element_type=F32))
    res = gate * outs[0] + (1.0 - gate) * outs[1]
    o_ref[...] = res.T.astype(o_ref.dtype)


def lax_dot_nt(a, b):
    return jax.lax.dot_general(a, b, _NT, preferred_element_type=F32)


@jax.jit
def pallas_gated_mix__mha_block__mha_block__prompt_kernel(
    A_x: jax.Array,
    A_wqkv: jax.Array,
    A_wo: jax.Array,
    B_x: jax.Array,
    B_wqkv: jax.Array,
    B_wo: jax.Array,
    gate_w: jax.Array,
):
    del B_x
    x = A_x.reshape(S, D)
    gw = gate_w.reshape(1, D)
    out = pl.pallas_call(
        _kernel,
        out_shape=jax.ShapeDtypeStruct((S, D), A_x.dtype),
        scratch_shapes=[
            pltpu.VMEM((2 * NG, S, 128), BF),
            pltpu.VMEM((2 * NG, S, 128), BF),
            pltpu.VMEM((NHEADS, 32, S), BF),
            pltpu.VMEM((S, BQ), F32),
            pltpu.VMEM((S, BQ), F32),
            pltpu.VMEM((8, BQ), F32),
            pltpu.VMEM((8, BQ), F32),
            pltpu.VMEM((NHEADS, 32, S), BF),
        ],
        compiler_params=pltpu.CompilerParams(vmem_limit_bytes=110 * 1024 * 1024),
    )(x, A_wqkv, A_wo, B_wqkv, B_wo, gw)
    return out.reshape(1, S, D)
```

```python
import math

import jax
import jax.numpy as jnp
import jax.experimental.pallas as pl
import jax.experimental.pallas.tpu as pltpu

S = 2048
D = 448
H = 16
DH = D // H
G = 4
NG = H // G
GW = G * DH
BQ = 512
KC = 128
NQ = S // BQ
NHEADS = 2 * H
NIT = NHEADS * NQ
UNROLL = 6
QSCALE = (DH ** -0.5) * math.log2(math.e)
BF = jnp.bfloat16
F32 = jnp.float32


def _dot(a, b):
    return jnp.dot(a, b, preferred_element_type=F32)


def _t(a):
    return a.astype(F32).T.astype(BF)


def _kernel(xt_hbm, wa_hbm, woa_hbm, wb_hbm, wob_hbm, gw_hbm, o_hbm,
            gw_ref,
            xt_v, wa_v, wb_v, wo_v, wt_v, xn_v, k_scr, qt_scr, vt_scr, s0, s1, m0, m1, ot_scr, g_scr, o_v, sems):
    RC = 512
    NR = S // RC
    c_wv = pltpu.make_async_copy(wa_hbm.at[:, 2 * D:3 * D], wa_v.at[:, 2 * D:3 * D], sems.at[0])
    c_x = [pltpu.make_async_copy(xt_hbm.at[:, r * RC:(r + 1) * RC], xt_v.at[:, r * RC:(r + 1) * RC],
                                 sems.at[1 + r]) for r in range(NR)]
    c_wqk = pltpu.make_async_copy(wa_hbm.at[:, 0:2 * D], wa_v.at[:, 0:2 * D], sems.at[5])
    c_wb = pltpu.make_async_copy(wb_hbm, wb_v, sems.at[6])
    c_woa = pltpu.make_async_copy(woa_hbm, wo_v.at[0:D], sems.at[7])
    c_wob = pltpu.make_async_copy(wob_hbm, wo_v.at[D:2 * D], sems.at[8])
    c_gw = pltpu.make_async_copy(gw_hbm, gw_ref, sems.at[14])
    for cp in (c_wv, c_x[0], c_wqk, c_x[1], c_gw, c_x[2], c_x[3], c_wb, c_woa, c_wob):
        cp.start()

    row = jax.lax.broadcasted_iota(jnp.int32, (32, RC), 0)

    def v_proj(b, wvt, r):
        cs = slice(r * RC, (r + 1) * RC)
        vt = _dot(wvt, xt_v[:, cs])
        for h in range(H):
            if h < H - 1:
                vh = vt[h * DH: h * DH + 32, :]
            else:
                vh = jnp.concatenate([vt[h * DH:, :], jnp.zeros((32 - DH, RC), F32)], axis=0)
            vt_scr[b * H + h, :, cs] = jnp.where(row == DH, 1.0, vh).astype(BF)

    def q_proj(b, wqt, r):
        cs = slice(r * RC, (r + 1) * RC)
        qt_scr[b, 0:D, cs] = (_dot(wqt, xt_v[:, cs]) * QSCALE).astype(BF)

    def xn_t(r):
        cs = slice(r * RC, (r + 1) * RC)
        xn_v[cs, :] = _t(xt_v[:, cs])

    c_wv.wait()
    c_x[0].wait()
    wvt = _t(wa_v[:, 2 * D:3 * D])
    v_proj(0, wvt, 0)
    xn_t(0)
    c_wqk.wait()
    c_x[1].wait()
    wqt = _t(wa_v[:, 0:D])
    q_proj(0, wqt, 0)
    v_proj(0, wvt, 1)
    q_proj(0, wqt, 1)
    xn_t(1)
    wt_v[0] = wvt
    wt_v[1] = wqt
    for cp in (c_gw, c_x[2], c_x[3], c_wb, c_woa, c_wob):
        cp.wait()
    wvt = wt_v[0]
    wqt = wt_v[1]
    for r in range(2, NR):
        v_proj(0, wvt, r)
        q_proj(0, wqt, r)
        xn_t(r)
    gl = _dot(jnp.broadcast_to(gw_ref[...].reshape(1, D), (16, D)), xt_v[...])[0:8, :]
    gate = 1.0 / (1.0 + jnp.exp(-gl))
    g_scr[0] = gate
    g_scr[1] = 1.0 - gate
    wk = jnp.concatenate([wa_v[:, D:2 * D], wb_v[:, D:2 * D]], axis=1)
    for r in range(NR):
        cs = slice(r * RC, (r + 1) * RC)
        kk = _dot(xn_v[cs, :], wk).astype(BF)
        kk = jnp.concatenate([kk, jnp.zeros((RC, 16), BF)], axis=1)
        for g in range(2 * NG):
            k_scr[g, cs, :] = kk[:, g * GW: g * GW + 128]
    wvt = _t(wb_v[:, 2 * D:3 * D])
    wqt = _t(wb_v[:, 0:D])
    for r in range(NR):
        v_proj(1, wvt, r)
        q_proj(1, wqt, r)
    for b in range(2):
        qt_scr[b, D:D + 16, :] = jnp.zeros((16, S), BF)

    srow = jax.lax.broadcasted_iota(jnp.int32, (128, BQ), 0)

    def step(itA, sA, mA, itB, sB, mB_ref, doA=True, doB=True):
        st = {}
        if doA:
            hA = itA // NQ
            qsA = pl.multiple_of((itA % NQ) * BQ, BQ)
            gA = hA // G
            bA = hA // H
            r0 = pl.multiple_of((gA % NG) * GW, 16)
            lo = (hA % G) * DH
            q = qt_scr[bA, pl.ds(r0, 128), pl.ds(qsA, BQ)]
            qm = jnp.where((srow >= lo) & (srow < lo + DH), q, jnp.zeros_like(q))
            st['m'] = None
        if doB:
            hB = itB // NQ
            qsB = pl.multiple_of((itB % NQ) * BQ, BQ)
            mm = jnp.tile(mB_ref[...], (KC // 8, 1))
            st['acc'] = jnp.zeros((32, BQ), F32)

        def a(c):
            kk = k_scr[gA, c * KC:(c + 1) * KC, :]
            s = _dot(kk, qm)
            sA[c * KC:(c + 1) * KC, :] = s
            sm = s[0:8]
            for r in range(1, KC // 8):
                sm = jnp.maximum(sm, s[r * 8:(r + 1) * 8])
            st['m'] = sm if st['m'] is None else jnp.maximum(st['m'], sm)

        def b(c):
            s = sB[c * KC:(c + 1) * KC, :]
            p = jnp.exp2(s - mm).astype(BF)
            st['acc'] = st['acc'] + _dot(vt_scr[hB, :, c * KC:(c + 1) * KC], p)

        for c in range(S // KC):
            if doA:
                a(c)
            if doB:
                b(c)
        if doA:
            mA[...] = jnp.broadcast_to(jnp.max(st['m'], axis=0, keepdims=True), (8, BQ))
        if doB:
            acc = st['acc']
            l = acc[DH:DH + 1, :]
            sc = g_scr[hB // H, 0:1, pl.ds(qsB, BQ)] / l
            ot_scr[pl.ds(pl.multiple_of(hB * 32, 32), 32), pl.ds(qsB, BQ)] = acc * sc

    bufs = [(s0, m0), (s1, m1)]

    def full(i, par):
        step(i, bufs[par][0], bufs[par][1], i - 1, bufs[1 - par][0], bufs[1 - par][1])

    step(0, s0, m0, None, None, None, True, False)
    ntrips = (NIT - 1) // UNROLL

    def body(j, c):
        for u in range(UNROLL):
            full(1 + j * UNROLL + u, (1 + u) % 2)
        return c

    jax.lax.fori_loop(0, ntrips, body, 0)
    for i in range(1 + ntrips * UNROLL, NIT):
        full(i, i % 2)

    out_copies = []

    def out_proj(r, parts=1):
        cs = slice(r * RC, (r + 1) * RC)
        oc = jnp.concatenate([ot_scr[h * 32:h * 32 + DH, cs] for h in range(NHEADS)],
                             axis=0).astype(BF)
        rows = D // parts
        for p in range(parts):
            rs = slice(p * rows, (p + 1) * rows)
            o_v[rs, cs] = _dot(wot[rs, :], oc).astype(o_v.dtype)
            cp = pltpu.make_async_copy(o_v.at[rs, cs], o_hbm.at[rs, cs], sems.at[9 + len(out_copies)])
            cp.start()
            out_copies.append(cp)

    wot = _t(wo_v[...])
    for r in range(NR - 1):
        out_proj(r)
    last = (NIT - 1) % 2
    step(None, None, None, NIT - 1, bufs[last][0], bufs[last][1], False, True)
    out_proj(NR - 1, parts=2)
    for cp in out_copies:
        cp.wait()


@jax.jit
def pallas_gated_mix__mha_block__mha_block__prompt_kernel(
    A_x: jax.Array,
    A_wqkv: jax.Array,
    A_wo: jax.Array,
    B_x: jax.Array,
    B_wqkv: jax.Array,
    B_wo: jax.Array,
    gate_w: jax.Array,
):
    del B_x
    xt = A_x.reshape(S, D).T
    any_spec = pl.BlockSpec(memory_space=pl.ANY)
    out_t = pl.pallas_call(
        _kernel,
        out_shape=jax.ShapeDtypeStruct((D, S), A_x.dtype),
        in_specs=[any_spec] * 6,
        out_specs=any_spec,
        scratch_shapes=[
            pltpu.VMEM((D,), BF),
            pltpu.VMEM((D, S), BF),
            pltpu.VMEM((D, 3 * D), BF),
            pltpu.VMEM((D, 3 * D), BF),
            pltpu.VMEM((2 * D, D), BF),
            pltpu.VMEM((2, D, D), BF),
            pltpu.VMEM((S, D), BF),
            pltpu.VMEM((2 * NG, S, 128), BF),
            pltpu.VMEM((2, D + 16, S), BF),
            pltpu.VMEM((NHEADS, 32, S), BF),
            pltpu.VMEM((S, BQ), F32),
            pltpu.VMEM((S, BQ), F32),
            pltpu.VMEM((8, BQ), F32),
            pltpu.VMEM((8, BQ), F32),
            pltpu.VMEM((NHEADS * 32, S), F32),
            pltpu.VMEM((2, 8, S), F32),
            pltpu.VMEM((D, S), BF),
            pltpu.SemaphoreType.DMA((15,)),
        ],
        compiler_params=pltpu.CompilerParams(vmem_limit_bytes=110 * 1024 * 1024),
    )(xt, A_wqkv, A_wo, B_wqkv, B_wo, gate_w)
    return out_t.T.reshape(1, S, D)
```

```python
import math

import jax
import jax.numpy as jnp
import jax.experimental.pallas as pl
import jax.experimental.pallas.tpu as pltpu

S = 2048
D = 448
H = 16
DH = D // H
G = 4
NG = H // G
GW = G * DH
BQ = 512
KC = 128
NQ = S // BQ
NHEADS = 2 * H
NIT = NHEADS * NQ
UNROLL = 6
NEW0 = 4
QSCALE = (DH ** -0.5) * math.log2(math.e)
BF = jnp.bfloat16
F32 = jnp.float32
U32 = jnp.uint32


def _dot(a, b):
    return jnp.dot(a, b, preferred_element_type=F32)


def _t(a):
    return a.astype(F32).T.astype(BF)


def _kernel(xt_hbm, wa_hbm, woa_hbm, wb_hbm, wob_hbm, gw_hbm, o_hbm,
            gw_ref,
            xt_v, wa_v, wb_v, wo_v, wt_v, xn_v, k_scr, qt_scr, vt_scr, s0, s1, m0, m1, ot_scr, g_scr, o_v, sems):
    RC = 512
    NR = S // RC
    c_wv = pltpu.make_async_copy(wa_hbm.at[:, 2 * D:3 * D], wa_v.at[:, 2 * D:3 * D], sems.at[0])
    c_x = [pltpu.make_async_copy(xt_hbm.at[:, r * RC:(r + 1) * RC], xt_v.at[:, r * RC:(r + 1) * RC],
                                 sems.at[1 + r]) for r in range(NR)]
    c_wq = pltpu.make_async_copy(wa_hbm.at[:, 0:512], wa_v.at[:, 0:512], sems.at[5])
    c_wk = pltpu.make_async_copy(wa_hbm.at[:, 512:2 * D], wa_v.at[:, 512:2 * D], sems.at[15])
    c_wb = pltpu.make_async_copy(wb_hbm, wb_v, sems.at[6])
    c_woa = pltpu.make_async_copy(woa_hbm, wo_v.at[0:D], sems.at[7])
    c_wob = pltpu.make_async_copy(wob_hbm, wo_v.at[D:2 * D], sems.at[8])
    c_gw = pltpu.make_async_copy(gw_hbm, gw_ref, sems.at[14])
    for cp in (c_wv, c_x[0], c_wq, c_x[1], c_gw, c_x[2], c_x[3], c_wk, c_wb, c_woa, c_wob):
        cp.start()

    row = jax.lax.broadcasted_iota(jnp.int32, (32, RC), 0)

    def v_proj(b, wvt, r):
        cs = slice(r * RC, (r + 1) * RC)
        vt = _dot(wvt, xt_v[:, cs])
        for h in range(H):
            if h < H - 1:
                vh = vt[h * DH: h * DH + 32, :]
            else:
                vh = jnp.concatenate([vt[h * DH:, :], jnp.zeros((32 - DH, RC), F32)], axis=0)
            vt_scr[b * H + h, :, cs] = pltpu.bitcast(jnp.where(row == DH, 1.0, vh).astype(BF), U32)

    def q_proj(b, wqt, r):
        cs = slice(r * RC, (r + 1) * RC)
        qt_scr[b, 0:D // 2, cs] = pltpu.bitcast((_dot(wqt, xt_v[:, cs]) * QSCALE).astype(BF), U32)

    def xn_t(r):
        cs = slice(r * RC, (r + 1) * RC)
        xn_v[r * RC // 2:(r + 1) * RC // 2, :] = pltpu.bitcast(_t(xt_v[:, cs]), U32)

    c_wv.wait()
    c_x[0].wait()
    wvt = _t(wa_v[:, 2 * D:3 * D])
    v_proj(0, wvt, 0)
    xn_t(0)
    c_wq.wait()
    c_x[1].wait()
    wqt = _t(wa_v[:, 0:D])
    q_proj(0, wqt, 0)
    v_proj(0, wvt, 1)
    q_proj(0, wqt, 1)
    xn_t(1)
    wt_v[0] = wvt
    wt_v[1] = wqt
    for cp in (c_gw, c_x[2], c_x[3], c_wk, c_wb):
        cp.wait()
    wvt = wt_v[0]
    wqt = wt_v[1]
    for r in range(2, NR):
        v_proj(0, wvt, r)
        q_proj(0, wqt, r)
        xn_t(r)
    gl = _dot(jnp.broadcast_to(gw_ref[...].reshape(1, D), (16, D)), xt_v[...])[0:8, :]
    gate = 1.0 / (1.0 + jnp.exp(-gl))
    g_scr[0] = gate
    g_scr[1] = 1.0 - gate
    wk = jnp.concatenate([wa_v[:, D:2 * D], wb_v[:, D:2 * D]], axis=1)
    for r in range(NR):
        cs = slice(r * RC, (r + 1) * RC)
        kk = _dot(pltpu.bitcast(xn_v[r * RC // 2:(r + 1) * RC // 2, :], BF), wk).astype(BF)
        kk = jnp.concatenate([kk, jnp.zeros((RC, 16), BF)], axis=1)
        for g in range(2 * NG):
            k_scr[g, r * RC // 2:(r + 1) * RC // 2, :] = pltpu.bitcast(kk[:, g * GW: g * GW + 128], U32)
    wvt = _t(wb_v[:, 2 * D:3 * D])
    wqt = _t(wb_v[:, 0:D])
    for r in range(NR):
        v_proj(1, wvt, r)
        q_proj(1, wqt, r)
    for b in range(2):
        qt_scr[b, D // 2:D // 2 + 8, :] = jnp.zeros((8, S), U32)

    srow = 2 * jax.lax.broadcasted_iota(jnp.int32, (64, BQ), 0)

    bufs = [(s0, m0), (s1, m1)]
    NC = S // KC
    HALF = NEW0

    def step(i, par, acc, doA=True, doB_old=True, doB_new=True):
        sA, mA = bufs[par]
        sN, mN = bufs[1 - par]
        m = None
        if doA:
            hA = i // NQ
            qsA = pl.multiple_of((i % NQ) * BQ, BQ)
            gA = hA // G
            bA = hA // H
            r0 = pl.multiple_of((gA % NG) * (GW // 2), 8)
            lo = (hA % G) * DH
            q = qt_scr[bA, pl.ds(r0, 64), pl.ds(qsA, BQ)]
            qm = pltpu.bitcast(jnp.where((srow >= lo) & (srow < lo + DH), q, jnp.zeros_like(q)), BF)

        def pv(item, s_ref, mm, c, acc):
            p = jnp.exp2(s_ref[c * KC:(c + 1) * KC, :] - mm).astype(BF)
            return acc + _dot(pltpu.bitcast(vt_scr[item // NQ, :, c * KC:(c + 1) * KC], BF), p)

        for c in range(NC):
            if c == HALF and doB_old:
                j = i - 2
                ot_scr[pl.ds(pl.multiple_of((j // NQ) * 32, 32), 32),
                       pl.ds(pl.multiple_of((j % NQ) * BQ, BQ), BQ)] = acc
            if c < HALF and doB_old:
                if c == 0:
                    mm = jnp.tile(mA[...], (KC // 8, 1))
            elif c >= HALF and doB_new:
                if c == HALF:
                    mm = jnp.tile(mN[...], (KC // 8, 1))
                    acc = jnp.zeros((32, BQ), F32)
            if doA:
                sc = _dot(pltpu.bitcast(k_scr[gA, c * KC // 2:(c + 1) * KC // 2, :], BF), qm)
            if c < HALF and doB_old:
                acc = pv(i - 2, sA, mm, c + NC - HALF, acc)
            elif c >= HALF and doB_new:
                acc = pv(i - 1, sN, mm, c - HALF, acc)
            if doA:
                sA[c * KC:(c + 1) * KC, :] = sc
                sm = sc[0:8]
                for r in range(1, KC // 8):
                    sm = jnp.maximum(sm, sc[r * 8:(r + 1) * 8])
                m = sm if m is None else jnp.maximum(m, sm)
        if doA:
            mA[...] = jnp.broadcast_to(jnp.max(m, axis=0, keepdims=True), (8, BQ))
        return acc

    acc = jnp.zeros((32, BQ), F32)
    acc = step(0, 0, acc, True, False, False)
    acc = step(1, 1, acc, True, False, True)
    ntrips = (NIT - 2) // UNROLL
    assert ntrips * UNROLL == NIT - 2

    def body(j, acc):
        for u in range(UNROLL):
            acc = step(2 + j * UNROLL + u, u % 2, acc)
        return acc

    c_woa.wait()
    c_wob.wait()
    acc = jax.lax.fori_loop(0, ntrips, body, acc)
    acc = step(NIT, NIT % 2, acc, False, True, True)

    out_copies = []

    def out_proj(r, parts=1):
        cs = slice(r * RC, (r + 1) * RC)
        heads = []
        for h in range(NHEADS):
            sc = g_scr[h // H, 0:1, cs] / ot_scr[h * 32 + DH:h * 32 + DH + 1, cs]
            heads.append(ot_scr[h * 32:h * 32 + DH, cs] * sc)
        oc = jnp.concatenate(heads, axis=0).astype(BF)
        rows = D // parts
        for p in range(parts):
            rs = slice(p * rows, (p + 1) * rows)
            o_v[rs, cs] = _dot(wot[rs, :], oc).astype(o_v.dtype)
            cp = pltpu.make_async_copy(o_v.at[rs, cs], o_hbm.at[rs, cs], sems.at[9 + len(out_copies)])
            cp.start()
            out_copies.append(cp)

    wot = _t(wo_v[...])
    for r in range(NR - 1):
        out_proj(r)
    step(NIT + 1, (NIT + 1) % 2, acc, False, True, False)
    out_proj(NR - 1, parts=2)
    for cp in out_copies:
        cp.wait()


@jax.jit
def pallas_gated_mix__mha_block__mha_block__prompt_kernel(
    A_x: jax.Array,
    A_wqkv: jax.Array,
    A_wo: jax.Array,
    B_x: jax.Array,
    B_wqkv: jax.Array,
    B_wo: jax.Array,
    gate_w: jax.Array,
):
    del B_x
    xt = A_x.reshape(S, D).T
    any_spec = pl.BlockSpec(memory_space=pl.ANY)
    out_t = pl.pallas_call(
        _kernel,
        out_shape=jax.ShapeDtypeStruct((D, S), A_x.dtype),
        in_specs=[any_spec] * 6,
        out_specs=any_spec,
        scratch_shapes=[
            pltpu.VMEM((D,), BF),
            pltpu.VMEM((D, S), BF),
            pltpu.VMEM((D, 3 * D), BF),
            pltpu.VMEM((D, 3 * D), BF),
            pltpu.VMEM((2 * D, D), BF),
            pltpu.VMEM((2, D, D), BF),
            pltpu.VMEM((S // 2, D), U32),
            pltpu.VMEM((2 * NG, S // 2, 128), U32),
            pltpu.VMEM((2, D // 2 + 8, S), U32),
            pltpu.VMEM((NHEADS, 16, S), U32),
            pltpu.VMEM((S, BQ), F32),
            pltpu.VMEM((S, BQ), F32),
            pltpu.VMEM((8, BQ), F32),
            pltpu.VMEM((8, BQ), F32),
            pltpu.VMEM((NHEADS * 32, S), F32),
            pltpu.VMEM((2, 8, S), F32),
            pltpu.VMEM((D, S), BF),
            pltpu.SemaphoreType.DMA((16,)),
        ],
        compiler_params=pltpu.CompilerParams(vmem_limit_bytes=110 * 1024 * 1024),
    )(xt, A_wqkv, A_wo, B_wqkv, B_wo, gate_w)
    return out_t.T.reshape(1, S, D)
```

```python
import math

import jax
import jax.numpy as jnp
import jax.experimental.pallas as pl
import jax.experimental.pallas.tpu as pltpu

S = 2048
D = 448
H = 16
DH = D // H
G = 4
NG = H // G
GW = G * DH
BQ = 512
KC = 128
NQ = S // BQ
NHEADS = 2 * H
NIT = NHEADS * NQ
UNROLL = 8
NEW0 = 4
QSCALE = (DH ** -0.5) * math.log2(math.e)
BF = jnp.bfloat16
F32 = jnp.float32
U32 = jnp.uint32


def _dot(a, b):
    return jnp.dot(a, b, preferred_element_type=F32)


def _t(a):
    return a.astype(F32).T.astype(BF)


def _kernel(xt_hbm, wa_hbm, woa_hbm, wb_hbm, wob_hbm, gw_hbm, o_hbm,
            gw_ref,
            xt_v, wa_v, wb_v, wo_v, wt_v, xn_v, k_scr, qt_scr, vt_scr, s0, s1, m0, m1, ot_scr, g_scr, o_v, sems):
    RC = 512
    NR = S // RC
    c_wv = pltpu.make_async_copy(wa_hbm.at[:, 2 * D:3 * D], wa_v.at[:, 2 * D:3 * D], sems.at[0])
    c_x = [pltpu.make_async_copy(xt_hbm.at[:, r * RC:(r + 1) * RC], xt_v.at[:, r * RC:(r + 1) * RC],
                                 sems.at[1 + r]) for r in range(NR)]
    c_wq = pltpu.make_async_copy(wa_hbm.at[:, 0:512], wa_v.at[:, 0:512], sems.at[5])
    c_wk = pltpu.make_async_copy(wa_hbm.at[:, 512:2 * D], wa_v.at[:, 512:2 * D], sems.at[16])
    c_wb = pltpu.make_async_copy(wb_hbm, wb_v, sems.at[6])
    c_woa = pltpu.make_async_copy(woa_hbm, wo_v.at[0:D], sems.at[7])
    c_wob = pltpu.make_async_copy(wob_hbm, wo_v.at[D:2 * D], sems.at[8])
    c_gw = pltpu.make_async_copy(gw_hbm, gw_ref, sems.at[17])
    for cp in (c_wv, c_x[0], c_wq, c_x[1], c_gw, c_x[2], c_x[3], c_wk, c_wb, c_woa, c_wob):
        cp.start()

    row = jax.lax.broadcasted_iota(jnp.int32, (32, RC), 0)

    def v_proj(b, wvt, r):
        cs = slice(r * RC, (r + 1) * RC)
        vt = _dot(wvt, xt_v[:, cs])
        for h in range(H):
            if h < H - 1:
                vh = vt[h * DH: h * DH + 32, :]
            else:
                vh = jnp.concatenate([vt[h * DH:, :], jnp.zeros((32 - DH, RC), F32)], axis=0)
            vt_scr[b * H + h, :, cs] = pltpu.bitcast(jnp.where(row == DH, 1.0, vh).astype(BF), U32)

    def q_proj(b, wqt, r):
        cs = slice(r * RC, (r + 1) * RC)
        qt_scr[b, 0:D // 2, cs] = pltpu.bitcast((_dot(wqt, xt_v[:, cs]) * QSCALE).astype(BF), U32)

    def xn_t(r):
        cs = slice(r * RC, (r + 1) * RC)
        xn_v[r * RC // 2:(r + 1) * RC // 2, :] = pltpu.bitcast(_t(xt_v[:, cs]), U32)

    c_wv.wait()
    c_x[0].wait()
    wvt = _t(wa_v[:, 2 * D:3 * D])
    v_proj(0, wvt, 0)
    xn_t(0)
    c_wq.wait()
    c_x[1].wait()
    wqt = _t(wa_v[:, 0:D])
    q_proj(0, wqt, 0)
    v_proj(0, wvt, 1)
    q_proj(0, wqt, 1)
    xn_t(1)
    wt_v[0] = wvt
    wt_v[1] = wqt
    for cp in (c_gw, c_x[2], c_x[3]):
        cp.wait()
    wvt = wt_v[0]
    wqt = wt_v[1]
    for r in range(2, NR):
        v_proj(0, wvt, r)
        q_proj(0, wqt, r)
        xn_t(r)
    gl = _dot(jnp.broadcast_to(gw_ref[...].reshape(1, D), (16, D)), xt_v[...])[0:8, :]
    gate = 1.0 / (1.0 + jnp.exp(-gl))
    g_scr[0] = gate
    g_scr[1] = 1.0 - gate
    c_wk.wait()
    c_wb.wait()
    wk = jnp.concatenate([wa_v[:, D:2 * D], wb_v[:, D:2 * D]], axis=1)
    for r in range(NR):
        cs = slice(r * RC, (r + 1) * RC)
        kk = _dot(pltpu.bitcast(xn_v[r * RC // 2:(r + 1) * RC // 2, :], BF), wk).astype(BF)
        kk = jnp.concatenate([kk, jnp.zeros((RC, 16), BF)], axis=1)
        for g in range(2 * NG):
            k_scr[g, r * RC // 2:(r + 1) * RC // 2, :] = pltpu.bitcast(kk[:, g * GW: g * GW + 128], U32)
    wvt = _t(wb_v[:, 2 * D:3 * D])
    wqt = _t(wb_v[:, 0:D])
    for r in range(NR):
        v_proj(1, wvt, r)
        q_proj(1, wqt, r)
    for b in range(2):
        qt_scr[b, D // 2:D // 2 + 8, :] = jnp.zeros((8, S), U32)

    srow = 2 * jax.lax.broadcasted_iota(jnp.int32, (64, BQ), 0)

    bufs = [(s0, m0), (s1, m1)]
    NC = S // KC
    HALF = NEW0

    def step(i, par, acc, doA=True, doB_old=True, doB_new=True):
        sA, mA = bufs[par]
        sN, mN = bufs[1 - par]
        m = None
        if doA:
            hA = i // NQ
            qsA = pl.multiple_of((i % NQ) * BQ, BQ)
            gA = hA // G
            bA = hA // H
            r0 = pl.multiple_of((gA % NG) * (GW // 2), 8)
            lo = (hA % G) * DH
            q = qt_scr[bA, pl.ds(r0, 64), pl.ds(qsA, BQ)]
            qm = pltpu.bitcast(jnp.where((srow >= lo) & (srow < lo + DH), q, jnp.zeros_like(q)), BF)

        def pv(item, s_ref, mm, c, acc):
            p = jnp.exp2(s_ref[c * KC:(c + 1) * KC, :] - mm).astype(BF)
            return acc + _dot(pltpu.bitcast(vt_scr[item // NQ, :, c * KC:(c + 1) * KC], BF), p)

        for c in range(NC):
            if c == HALF and doB_old:
                j = i - 2
                ot_scr[pl.ds(pl.multiple_of((j // NQ) * 32, 32), 32),
                       pl.ds(pl.multiple_of((j % NQ) * BQ, BQ), BQ)] = acc
            if c < HALF and doB_old:
                if c == 0:
                    mm = jnp.tile(mA[...], (KC // 8, 1))
            elif c >= HALF and doB_new:
                if c == HALF:
                    mm = jnp.tile(mN[...], (KC // 8, 1))
                    acc = jnp.zeros((32, BQ), F32)
            if doA:
                sc = _dot(pltpu.bitcast(k_scr[gA, c * KC // 2:(c + 1) * KC // 2, :], BF), qm)
            if c < HALF and doB_old:
                acc = pv(i - 2, sA, mm, c + NC - HALF, acc)
            elif c >= HALF and doB_new:
                acc = pv(i - 1, sN, mm, c - HALF, acc)
            if doA:
                sA[c * KC:(c + 1) * KC, :] = sc
                sm = sc[0:8]
                for r in range(1, KC // 8):
                    sm = jnp.maximum(sm, sc[r * 8:(r + 1) * 8])
                m = sm if m is None else jnp.maximum(m, sm)
        if doA:
            mA[...] = jnp.broadcast_to(jnp.max(m, axis=0, keepdims=True), (8, BQ))
        return acc

    acc = jnp.zeros((32, BQ), F32)
    acc = step(0, 0, acc, True, False, False)
    acc = step(1, 1, acc, True, False, True)
    ntrips = (NIT - 2) // UNROLL

    def body(j, acc):
        for u in range(UNROLL):
            acc = step(2 + j * UNROLL + u, u % 2, acc)
        return acc

    c_woa.wait()
    c_wob.wait()
    acc = jax.lax.fori_loop(0, ntrips, body, acc)
    for i in range(2 + ntrips * UNROLL, NIT):
        acc = step(i, i % 2, acc)
    acc = step(NIT, NIT % 2, acc, False, True, True)

    out_copies = []

    def out_proj(r, parts=1):
        cs = slice(r * RC, (r + 1) * RC)
        heads = []
        for h in range(NHEADS):
            sc = g_scr[h // H, 0:1, cs] / ot_scr[h * 32 + DH:h * 32 + DH + 1, cs]
            heads.append(ot_scr[h * 32:h * 32 + DH, cs] * sc)
        oc = jnp.concatenate(heads, axis=0).astype(BF)
        rows = D // parts
        for p in range(parts):
            rs = slice(p * rows, (p + 1) * rows)
            o_v[rs, cs] = _dot(wot[rs, :], oc).astype(o_v.dtype)
            cp = pltpu.make_async_copy(o_v.at[rs, cs], o_hbm.at[rs, cs], sems.at[9 + len(out_copies)])
            cp.start()
            out_copies.append(cp)

    wot = _t(wo_v[...])
    for r in range(NR - 1):
        out_proj(r)
    step(NIT + 1, (NIT + 1) % 2, acc, False, True, False)
    out_proj(NR - 1, parts=4)
    for cp in out_copies:
        cp.wait()


@jax.jit
def pallas_gated_mix__mha_block__mha_block__prompt_kernel(
    A_x: jax.Array,
    A_wqkv: jax.Array,
    A_wo: jax.Array,
    B_x: jax.Array,
    B_wqkv: jax.Array,
    B_wo: jax.Array,
    gate_w: jax.Array,
):
    del B_x
    xt = A_x.reshape(S, D).T
    any_spec = pl.BlockSpec(memory_space=pl.ANY)
    out_t = pl.pallas_call(
        _kernel,
        out_shape=jax.ShapeDtypeStruct((D, S), A_x.dtype),
        in_specs=[any_spec] * 6,
        out_specs=any_spec,
        scratch_shapes=[
            pltpu.VMEM((D,), BF),
            pltpu.VMEM((D, S), BF),
            pltpu.VMEM((D, 3 * D), BF),
            pltpu.VMEM((D, 3 * D), BF),
            pltpu.VMEM((2 * D, D), BF),
            pltpu.VMEM((2, D, D), BF),
            pltpu.VMEM((S // 2, D), U32),
            pltpu.VMEM((2 * NG, S // 2, 128), U32),
            pltpu.VMEM((2, D // 2 + 8, S), U32),
            pltpu.VMEM((NHEADS, 16, S), U32),
            pltpu.VMEM((S, BQ), F32),
            pltpu.VMEM((S, BQ), F32),
            pltpu.VMEM((8, BQ), F32),
            pltpu.VMEM((8, BQ), F32),
            pltpu.VMEM((NHEADS * 32, S), F32),
            pltpu.VMEM((2, 8, S), F32),
            pltpu.VMEM((D, S), BF),
            pltpu.SemaphoreType.DMA((18,)),
        ],
        compiler_params=pltpu.CompilerParams(vmem_limit_bytes=110 * 1024 * 1024),
    )(xt, A_wqkv, A_wo, B_wqkv, B_wo, gate_w)
    return out_t.T.reshape(1, S, D)
```
